```python
import os as _os
_os.environ.setdefault("JAX_PLATFORMS", "cpu")
import jax
import jax.numpy as jnp

def _softmax(x, axis=-1):
    return jax.nn.softmax(x, axis=axis)
def _gelu(x):
    return jax.nn.gelu(x, approximate=True)
def _silu(x):
    return jax.nn.silu(x)
def _sigmoid(x):
    return jax.nn.sigmoid(x)
def _layernorm(x, axis=-1, eps=1e-5):
    m = jnp.mean(x, axis=axis, keepdims=True)
    v = jnp.var(x, axis=axis, keepdims=True)
    return (x - m) / jnp.sqrt(v + eps)
def _scatter_add(tgt, idx, src, axis=0):
    return tgt.at[idx].add(src)
def _segment_sum(src, seg, n):
    return jax.ops.segment_sum(src, seg, n)
class _Rng:
    def __init__(self, key):
        self._k = key
    def _next(self):
        self._k, sub = jax.random.split(self._k)
        return sub
    def normal(self, shape):
        return jax.random.normal(self._next(), shape, dtype=jnp.bfloat16)
    def randint(self, lo, hi, shape):
        return jax.random.randint(self._next(), shape, lo, hi, dtype=jnp.int32)
    def uniform(self, shape, lo=0.0, hi=1.0):
        return jax.random.uniform(self._next(), shape, jnp.bfloat16, lo, hi)
    def permutation(self, n):
        return jax.random.permutation(self._next(), n)


kernel_name = 'gated_mix__mha_block_cached__swiglu_ffn__decode'

def setup_inputs():
    _rng = _Rng(jax.random.key(int.from_bytes(__import__("os").urandom(4), "little")))
    _w = (lambda a: (lambda t: t.astype(jnp.bfloat16) if jnp.issubdtype(t.dtype, jnp.floating) else t)(jnp.asarray(a)))
    def _A_setup():
        B, Sq, D = 4, 1, 512
        H, Sk, Dh = 32, 4096, 128
        return {
            "x": _w((lambda *s: _rng.normal(s) * 0.05)(B, Sq, D)),
            "k_cache": _w((lambda *s: _rng.normal(s) * 3.2)(B, H, Sk, Dh)),
            "v_cache": _w((lambda *s: _rng.normal(s) * 0.4)(B, H, Sk, Dh)),
            "wq": _w((lambda *s: _rng.normal(s) * 3.2)(D, H * Dh) * (D ** -0.5)),
            "wo": _w((lambda *s: _rng.normal(s) * 0.4)(H * Dh, D) * ((H * Dh) ** -0.5)),
        }
    _A_in = _A_setup()

    def _B_setup():
        B, S, D, F = 4, 1, 512, 1376
        return {
            "x": _w((lambda *s: _rng.normal(s) * 0.05)(B, S, D)),
            "w_gate": _w((lambda *s: _rng.normal(s) * 0.05)(D, F)),
            "w_up": _w((lambda *s: _rng.normal(s) * 0.05)(D, F)),
            "w_down": _w((lambda *s: _rng.normal(s) * 0.05)(F, D)),
        }
    _B_in = _B_setup()

    return {
        "A_x": _A_in["x"],
        "A_k_cache": _A_in["k_cache"],
        "A_v_cache": _A_in["v_cache"],
        "A_wq": _A_in["wq"],
        "A_wo": _A_in["wo"],
        "B_x": _B_in["x"],
        "B_w_gate": _B_in["w_gate"],
        "B_w_up": _B_in["w_up"],
        "B_w_down": _B_in["w_down"],
        "gate_w": _w((lambda *s: _rng.normal(s) * 0.05)(512) * 16.0),
    }

def reference(A_x, A_k_cache, A_v_cache, A_wq, A_wo, B_x, B_w_gate, B_w_up, B_w_down, gate_w):
    def _A_ref(x, k_cache, v_cache, wq, wo):
        B, Sq, D = x.shape
        H, Dh = 32, 128
        q = (lambda x, *d: x.transpose(*d))((x @ wq).reshape(B, Sq, H, Dh), 0, 2, 1, 3)
        scores = jnp.einsum("bhqd,bhkd->bhqk", q, k_cache) * (Dh ** -0.5)
        p = _softmax(scores, axis=-1)
        o = jnp.einsum("bhqk,bhkd->bhqd", p, v_cache)
        return (lambda x, *d: x.transpose(*d))(o, 0, 2, 1, 3).reshape(B, Sq, H * Dh) @ wo

    def _B_ref(x, w_gate, w_up, w_down):
        g = _silu(x @ w_gate)
        u = x @ w_up
        return (g * u) @ w_down

    x = A_x
    g = _sigmoid((x * gate_w).sum(-1, keepdims=True))
    a = _A_ref(x, A_k_cache, A_v_cache, A_wq, A_wo)
    b = _B_ref(x, B_w_gate, B_w_up, B_w_down)
    return g * a + (1 - g) * b
```

```python
import functools
import jax, jax.numpy as jnp, numpy as np
from jax import lax
from jax.experimental import pallas as pl
from jax.experimental.pallas import tpu as pltpu

B, D_MODEL, H, SK, DH, FF = 4, 512, 32, 4096, 128, 1376
NS = 16
NW = B * H // NS
CH = 128
NC = SK // CH
f32, bf16 = jnp.float32, jnp.bfloat16
NT = (((1,), (1,)), ((), ()))

def make(name="kern", D=5, order="kv", interleave=True, nobounds=False, wq_mode="16x1024", flags=None):
    def kern(x_hbm, k_hbm, v_hbm, wq_hbm, wo_hbm, wg_hbm, wu_hbm, wd_hbm, gw_hbm, o_hbm,
             kv, wq_v, wo_v, wg_v, wu_v, wd_v, x_v, gw_v, q_v, o_v, ring_sem, w_sem):
        def kv_copy(t, slot, j):
            isv, r = j // NS, j % NS
            wave, c = t // NC, t % NC
            src = (k_hbm, v_hbm)[isv]
            s = (r % 4) * 4 + r // 4
            return pltpu.make_async_copy(src.at[s, wave, pl.ds(pl.multiple_of(c * CH, CH), CH), :], kv.at[slot, j], ring_sem.at[slot])
        rows_by_addr = sorted(range(NS), key=lambda r: (r % 4) * 4 + r // 4)
        if order == "kv":
            issue = [r for r in rows_by_addr] + [NS + r for r in rows_by_addr]
        else:
            issue = [x for r in rows_by_addr for x in (r, NS + r)]
        def start_group(t, slot, lo=0, hi=2 * NS):
            for n in range(lo, hi):
                kv_copy(t, slot, issue[n]).start(priority=n % 2)
        def wait_group(slot):
            pltpu.make_async_copy(kv.at[slot], kv.at[slot], ring_sem.at[slot]).wait()

        def start_rows(src, dst, sem, nrows, step=32):
            n = nrows // step
            def body(i, _):
                for u in range(2):
                    r0 = pl.multiple_of((i + u * (n // 2)) * step, step)
                    pltpu.make_async_copy(src.at[pl.ds(r0, step), :], dst.at[pl.ds(r0, step), :], sem).start(priority=u)
            lax.fori_loop(0, n // 2, body, None)
            if n % 2:
                r0 = (n - 1) * step
                pltpu.make_async_copy(src.at[pl.ds(r0, step), :], dst.at[pl.ds(r0, step), :], sem).start()
        def wait_all(dst, sem):
            pltpu.make_async_copy(dst, dst, sem).wait()

        def wq_body(i, _):
            r0 = pl.multiple_of(i * 16, 16)
            for u in range(4):
                pltpu.make_async_copy(wq_hbm.at[pl.ds(r0, 16), pl.ds(u * 1024, 1024)], wq_v.at[pl.ds(r0, 16), pl.ds(u * 1024, 1024)], w_sem.at[0]).start(priority=u % 2)
        lax.fori_loop(0, D_MODEL // 16, wq_body, None)
        cx = pltpu.make_async_copy(x_hbm, x_v, w_sem.at[1]); cx.start()
        cg = pltpu.make_async_copy(gw_hbm, gw_v, w_sem.at[1]); cg.start(priority=1)
        start_rows(wg_hbm, wg_v, w_sem.at[2], FF)
        start_rows(wu_hbm, wu_v, w_sem.at[2], FF)
        cx.wait(); cg.wait()
        wait_all(wq_v, w_sem.at[0])

        row = lax.broadcasted_iota(jnp.int32, (NS, DH), 0)
        xf = x_v[...].astype(f32)
        row_d = lax.broadcasted_iota(jnp.int32, (NS, D_MODEL), 0)
        x16f = jnp.broadcast_to(xf[0:1], (NS, D_MODEL))
        for b in range(1, B):
            x16f = jnp.where(row_d % B == b, jnp.broadcast_to(xf[b:b + 1], (NS, D_MODEL)), x16f)
        x16 = x16f.astype(bf16)
        gwf = gw_v[...].astype(f32)
        gl = x16f[:, 0:128] * gwf[0:1]
        for j in range(1, 4):
            gl = gl + x16f[:, j * 128:(j + 1) * 128] * gwf[j:j + 1]
        gate = jax.nn.sigmoid(jnp.sum(gl, axis=-1, keepdims=True))

        start_rows(wd_hbm, wd_v, w_sem.at[3], FF)
        for i in range(NW):
            qi = None
            for j in range(4):
                c0 = (j * NW + i) * DH
                rj = jnp.dot(x16, wq_v[:, c0:c0 + DH], preferred_element_type=f32)
                qi = rj if qi is None else jnp.where(row // 4 == j, rj, qi)
            q_v[i] = qi.astype(bf16)
        start_rows(wo_hbm, wo_v, w_sem.at[4], H * DH)
        wait_all(wg_v, w_sem.at[2]); wait_all(wu_v, w_sem.at[2])
        hg = lax.dot_general(x16, wg_v[...], NT, preferred_element_type=f32)
        start_group(0, 0)
        hu = lax.dot_general(x16, wu_v[...], NT, preferred_element_type=f32)
        hh = (hg * jax.nn.sigmoid(hg) * hu).astype(bf16)
        start_group(1, 1)
        wait_all(wd_v, w_sem.at[3])
        ffn = jnp.dot(hh, wd_v[...], preferred_element_type=f32)
        for g in range(2, D - 1):
            start_group(g, g)
        wait_all(wo_v, w_sem.at[4])

        c_exp = np.float32(DH ** -0.5)
        T = NW * NC

        def step(t, carry, prefetch):
            slot, pslot, m, l, acc, a16 = carry
            wave, c = t // NC, t % NC
            wait_group(slot)
            q = q_v[wave]
            s = None
            for r in range(NS):
                if prefetch and interleave: start_group(t + D - 1, pslot, r, r + 1)
                sr = lax.dot_general(q, kv[slot, r], NT, preferred_element_type=f32)
                s = sr if s is None else jnp.where(row == r, sr, s)
            if prefetch and not interleave: start_group(t + D - 1, pslot)
            s = s * c_exp
            m_new = jnp.maximum(m, jnp.max(s, axis=-1, keepdims=True))
            alpha = jnp.exp(m - m_new)
            p = jnp.exp(s - m_new)
            l = alpha * l + p
            pb = p.astype(bf16)
            pv = None
            for r in range(NS):
                if prefetch and interleave: start_group(t + D - 1, pslot, NS + r, NS + r + 1)
                o = jnp.dot(pb, kv[slot, NS + r], preferred_element_type=f32)
                pv = o if pv is None else jnp.where(row == r, o, pv)
            acc = alpha * acc + pv

            def fin(m, l, acc, a16):
                o16 = (acc / jnp.sum(l, axis=-1, keepdims=True))
                for j in range(4):
                    oj = jnp.where(row // 4 == j, o16, 0.0).astype(bf16)
                    r0 = pl.multiple_of((j * NW + wave) * DH, DH)
                    a16 = a16 + jnp.dot(oj, wo_v[pl.ds(r0, DH), :], preferred_element_type=f32)
                return jnp.full_like(m, -jnp.inf), jnp.zeros_like(l), jnp.zeros_like(acc), a16
            m, l, acc, a16 = lax.cond(c == NC - 1, fin, lambda *a: a, m_new, l, acc, a16)
            nslot = jnp.where(slot == D - 1, 0, slot + 1)
            return nslot, slot, m, l, acc, a16

        carry = (jnp.int32(0), jnp.int32(D - 1), jnp.full((NS, 1), -jnp.inf, f32), jnp.zeros((NS, DH), f32),
                 jnp.zeros((NS, DH), f32), jnp.zeros((NS, D_MODEL), f32))
        carry = lax.fori_loop(0, T - (D - 1), functools.partial(step, prefetch=True), carry)
        carry = lax.fori_loop(T - (D - 1), T, functools.partial(step, prefetch=False), carry)
        a16 = carry[-1]
        a8 = a16[0:8] + a16[8:16]
        a8 = a8 + pltpu.roll(a8, 4, 0)
        out = gate[0:8] * a8 + (1.0 - gate[0:8]) * ffn[0:8]
        o_v[...] = out[0:4].astype(bf16)
        co = pltpu.make_async_copy(o_v, o_hbm, w_sem.at[0]); co.start(); co.wait()

    def f(A_x, A_k_cache, A_v_cache, A_wq, A_wo, B_x, B_w_gate, B_w_up, B_w_down, gate_w):
        h = pl.BlockSpec(memory_space=pltpu.HBM)
        out = pl.pallas_call(
            kern, out_shape=jax.ShapeDtypeStruct((B, D_MODEL), bf16), in_specs=[h] * 9, out_specs=h,
            scratch_shapes=[
                pltpu.VMEM((D, 2 * NS, CH, DH), bf16),
                pltpu.VMEM((D_MODEL, H * DH), bf16), pltpu.VMEM((H * DH, D_MODEL), bf16),
                pltpu.VMEM((FF, D_MODEL), bf16), pltpu.VMEM((FF, D_MODEL), bf16), pltpu.VMEM((FF, D_MODEL), bf16),
                pltpu.VMEM((B, D_MODEL), bf16), pltpu.VMEM((4, 128), bf16),
                pltpu.VMEM((NW, NS, DH), bf16), pltpu.VMEM((B, D_MODEL), bf16),
                pltpu.SemaphoreType.DMA((D,)), pltpu.SemaphoreType.DMA((5,)),
            ],
            compiler_params=pltpu.CompilerParams(vmem_limit_bytes=64 * 1024 * 1024, disable_bounds_checks=nobounds, flags=flags),
            name=name,
        )(A_x.reshape(B, D_MODEL), A_k_cache.reshape(NS, NW, SK, DH), A_v_cache.reshape(NS, NW, SK, DH),
          A_wq, A_wo, B_w_gate.T, B_w_up.T, B_w_down, gate_w.reshape(4, 128))
        return out.reshape(B, 1, D_MODEL)
    return f


_impl = make(name="gated_mix_decode", D=5)


@jax.jit
def pallas_gated_mix__mha_block_cached__swiglu_ffn__decode_kernel(
    A_x, A_k_cache, A_v_cache, A_wq, A_wo, B_x, B_w_gate, B_w_up, B_w_down, gate_w
):
    return _impl(A_x, A_k_cache, A_v_cache, A_wq, A_wo, B_x, B_w_gate, B_w_up, B_w_down, gate_w)
```

```python
import functools

import jax
import jax.experimental.pallas as pl
import jax.experimental.pallas.tpu as pltpu
import jax.numpy as jnp
import numpy as np
from jax import lax

BATCH, D_MODEL, HEADS, SEQ, D_HEAD, D_FF = 4, 512, 32, 4096, 128, 1376

STREAMS = 16
WAVES = BATCH * HEADS // STREAMS
HEAD_GROUPS = STREAMS // BATCH
KEYS = 128
CHUNKS = SEQ // KEYS
STEPS = WAVES * CHUNKS
SLOTS = 6

W_ROWS = 32
FF_BLOCKS = D_FF // W_ROWS
FF_EDGES = (0,) + tuple(range(D_FF % 128, D_FF + 1, 128))
FF_TILES = tuple(zip(FF_EDGES[:-1], FF_EDGES[1:]))
DOWN_PIECES = ((0, 31, 11), (31, 39, 3), (39, FF_BLOCKS, 1))
DOWN_ALTERNATING = 25

_CONTRACT_LAST = (((1,), (1,)), ((), ()))


def _dot(a, b):
    return jnp.dot(a, b, preferred_element_type=jnp.float32)


def _dot_t(a, b):
    return lax.dot_general(a, b, _CONTRACT_LAST, preferred_element_type=jnp.float32)


def _wait_filled(buf, sem):
    pltpu.make_async_copy(buf, buf, sem).wait()


def _start_rows(src, dst, block, sem, priority):
    row0 = block * W_ROWS
    if not isinstance(row0, int):
        row0 = pl.multiple_of(row0, W_ROWS)
    rows = pl.ds(row0, W_ROWS)
    pltpu.make_async_copy(src.at[rows, :], dst.at[rows, :], sem).start(priority=priority)


def _kernel(
    x_hbm, k_hbm, v_hbm, wq_hbm, wo_hbm, wgate_t_hbm, wup_t_hbm, wdown_hbm, gate_w_hbm,
    out_hbm,
    kv_buf, wq_buf, wo_buf, wgu_buf, wdown_buf, x_buf, gate_w_buf, q_buf, out_buf,
    kv_sems, w_sems,
):
    f32, bf16 = jnp.float32, jnp.bfloat16
    sem_a, sem_b, sem_c = (w_sems.at[i] for i in range(3))

    def start_kv(step, slot, n):
        is_v, stream = divmod(n, STREAMS)
        batch, head_group = divmod(stream, HEAD_GROUPS)
        wave = lax.div(step, CHUNKS)
        key0 = pl.multiple_of(lax.rem(step, CHUNKS) * KEYS, KEYS)
        pltpu.make_async_copy(
            (k_hbm, v_hbm)[is_v].at[stream, wave, pl.ds(key0, KEYS), :],
            kv_buf.at[slot, is_v, head_group * BATCH + batch],
            kv_sems.at[slot],
        ).start(priority=1 - n % 2)

    def projection_copies(i, _, wo_priority):
        for j in range(8):
            block = j * 16 + i
            rows = pl.ds(pl.multiple_of(lax.div(block, 2) * 8, 8), 8)
            cols = pl.ds(pl.multiple_of(lax.rem(block, 2) * 2048, 2048), 2048)
            pltpu.make_async_copy(
                wq_hbm.at[rows, cols], wq_buf.at[rows, cols], sem_a
            ).start(priority=1)
            _start_rows(wo_hbm, wo_buf, block, sem_b, wo_priority)

    lax.fori_loop(0, 2, functools.partial(projection_copies, wo_priority=1), None)
    lax.fori_loop(2, 16, functools.partial(projection_copies, wo_priority=0), None)

    x_copy = pltpu.make_async_copy(x_hbm, x_buf, kv_sems.at[SLOTS - 1])
    gate_w_copy = pltpu.make_async_copy(gate_w_hbm, gate_w_buf, kv_sems.at[SLOTS - 2])
    x_copy.start()
    gate_w_copy.start()

    def ffn_copies(i, _):
        block = lax.rem(i * 11, FF_BLOCKS)
        _start_rows(wgate_t_hbm, wgu_buf.at[0], block, sem_c, 1)
        _start_rows(wup_t_hbm, wgu_buf.at[1], block, sem_c, 0)

    lax.fori_loop(0, FF_BLOCKS, ffn_copies, None)

    x_copy.wait()
    gate_w_copy.wait()
    row = lax.broadcasted_iota(jnp.int32, (STREAMS, D_HEAD), 0)
    head_group = row >> 2
    batch = lax.broadcasted_iota(jnp.int32, (STREAMS, D_MODEL), 0) & (BATCH - 1)
    x = x_buf[...].astype(f32)
    x_rows = jnp.broadcast_to(x[0:1], (STREAMS, D_MODEL))
    for b in range(1, BATCH):
        x_rows = jnp.where(batch == b, jnp.broadcast_to(x[b:b + 1], x_rows.shape), x_rows)
    x_rows_bf16 = x_rows.astype(bf16)

    gate_w = gate_w_buf[...].astype(f32)
    gate_terms = x_rows[:, 0:128] * gate_w[0:1]
    for j in range(1, D_MODEL // 128):
        gate_terms = gate_terms + x_rows[:, j * 128:(j + 1) * 128] * gate_w[j:j + 1]
    gate = jax.nn.sigmoid(jnp.sum(gate_terms, axis=-1, keepdims=True))

    def fill_slot(step, _):
        for n in range(2 * STREAMS):
            start_kv(step, step, n)

    def fill_slot_and_project(step, _):
        fill_slot(step, None)
        for u in range(2):
            wave = 2 * step + u
            q = None
            for j in range(HEAD_GROUPS):
                cols = pl.ds(pl.multiple_of((j * WAVES + wave) * D_HEAD, D_HEAD), D_HEAD)
                q_j = _dot(x_rows_bf16, wq_buf[:, cols])
                q = q_j if q is None else jnp.where(head_group == j, q_j, q)
            q_buf[wave] = q.astype(bf16)

    _wait_filled(wq_buf, sem_a)
    lax.fori_loop(0, WAVES // 2, fill_slot_and_project, None)
    lax.fori_loop(WAVES // 2, SLOTS - 1, fill_slot, None)

    _wait_filled(wgu_buf, sem_c)
    hidden = []
    for lo, hi in FF_TILES:
        g = _dot_t(x_rows_bf16, wgu_buf[0, lo:hi, :])
        u = _dot_t(x_rows_bf16, wgu_buf[1, lo:hi, :])
        hidden.append((g * jax.nn.sigmoid(g) * u).astype(bf16))
    _wait_filled(wo_buf, sem_b)

    lowest = np.finfo(np.float32).min

    def attend(step, carry, prefetch):
        slot, free_slot, m, l, acc, attn = carry
        wave = lax.div(step, CHUNKS)
        _wait_filled(kv_buf.at[slot], kv_sems.at[slot])

        q = q_buf[wave]
        s = None
        for r in range(STREAMS):
            if prefetch:
                start_kv(step + SLOTS - 1, free_slot, r)
            s_r = _dot_t(q, kv_buf[slot, 0, r])
            s = s_r if s is None else jnp.where(row == r, s_r, s)
        s = s * np.float32(D_HEAD ** -0.5)

        m_new = jnp.maximum(m, jnp.max(s, axis=-1, keepdims=True))
        alpha = jnp.exp(m - m_new)
        p = jnp.exp(s - m_new)
        l = alpha * l + p
        p = p.astype(bf16)

        pv = None
        for r in range(STREAMS):
            if prefetch:
                start_kv(step + SLOTS - 1, free_slot, STREAMS + r)
            pv_r = _dot(p, kv_buf[slot, 1, r])
            pv = pv_r if pv is None else jnp.where(row == r, pv_r, pv)
        acc = alpha * acc + pv

        def finish_wave(m, l, acc, attn):
            o = acc / jnp.sum(l, axis=-1, keepdims=True)
            for j in range(HEAD_GROUPS):
                rows = pl.ds(pl.multiple_of((j * WAVES + wave) * D_HEAD, D_HEAD), D_HEAD)
                o_j = jnp.where(head_group == j, o, 0.0).astype(bf16)
                attn = attn + _dot(o_j, wo_buf[rows, :])
            return jnp.full_like(m, lowest), jnp.zeros_like(l), jnp.zeros_like(acc), attn

        state = lax.cond(
            lax.rem(step, CHUNKS) == CHUNKS - 1,
            finish_wave, lambda *state: state, m_new, l, acc, attn,
        )
        next_slot = jnp.where(slot == SLOTS - 1, 0, slot + 1)
        return (next_slot, slot) + tuple(state)

    carry = (
        jnp.int32(0),
        jnp.int32(SLOTS - 1),
        jnp.full((STREAMS, 1), lowest, f32),
        jnp.zeros((STREAMS, D_HEAD), f32),
        jnp.zeros((STREAMS, D_HEAD), f32),
        jnp.zeros((STREAMS, D_MODEL), f32),
    )
    last_prefetch = STEPS - (SLOTS - 1)
    carry = lax.fori_loop(0, last_prefetch, functools.partial(attend, prefetch=True), carry)

    down_sems = (sem_a, sem_b, sem_c)
    for (lo, hi, stride), sem in zip(DOWN_PIECES, down_sems):
        for i in range(hi - lo):
            n = lo + i
            priority = 1 - n % 2 if n < DOWN_ALTERNATING else 1
            _start_rows(wdown_hbm, wdown_buf, lo + (i * stride) % (hi - lo), sem, priority)

    carry = lax.fori_loop(last_prefetch, STEPS, functools.partial(attend, prefetch=False), carry)

    attn = carry[-1]
    attn = attn[0:8] + attn[8:16]
    attn = attn + pltpu.roll(attn, BATCH, 0)

    ffn = None
    for (lo, hi, _), sem in zip(DOWN_PIECES, down_sems):
        _wait_filled(wdown_buf.at[pl.ds(lo * W_ROWS, (hi - lo) * W_ROWS), :], sem)
        for h, (r0, r1) in zip(hidden, FF_TILES):
            if lo * W_ROWS <= r0 and r1 <= hi * W_ROWS:
                part = _dot(h, wdown_buf[r0:r1, :])
                ffn = part if ffn is None else ffn + part

    out = gate[0:8] * attn + (1.0 - gate[0:8]) * ffn[0:8]
    out_buf[...] = out[0:BATCH].astype(bf16)
    out_copy = pltpu.make_async_copy(out_buf, out_hbm, sem_a)
    out_copy.start()
    out_copy.wait()


@jax.jit
def pallas_gated_mix__mha_block_cached__swiglu_ffn__decode_kernel(
    A_x: jax.Array,
    A_k_cache: jax.Array,
    A_v_cache: jax.Array,
    A_wq: jax.Array,
    A_wo: jax.Array,
    B_x: jax.Array,
    B_w_gate: jax.Array,
    B_w_up: jax.Array,
    B_w_down: jax.Array,
    gate_w: jax.Array,
):
    del B_x
    bf16 = jnp.bfloat16
    hbm = pl.BlockSpec(memory_space=pltpu.HBM)
    out = pl.pallas_call(
        _kernel,
        out_shape=jax.ShapeDtypeStruct((BATCH, D_MODEL), bf16),
        in_specs=[hbm] * 9,
        out_specs=hbm,
        scratch_shapes=[
            pltpu.VMEM((SLOTS, 2, STREAMS, KEYS, D_HEAD), bf16),
            pltpu.VMEM((D_MODEL, HEADS * D_HEAD), bf16),
            pltpu.VMEM((HEADS * D_HEAD, D_MODEL), bf16),
            pltpu.VMEM((2, D_FF, D_MODEL), bf16),
            pltpu.VMEM((D_FF, D_MODEL), bf16),
            pltpu.VMEM((BATCH, D_MODEL), bf16),
            pltpu.VMEM((D_MODEL // 128, 128), bf16),
            pltpu.VMEM((WAVES, STREAMS, D_HEAD), bf16),
            pltpu.VMEM((BATCH, D_MODEL), bf16),
            pltpu.SemaphoreType.DMA((SLOTS,)),
            pltpu.SemaphoreType.DMA((3,)),
        ],
        compiler_params=pltpu.CompilerParams(
            vmem_limit_bytes=32 * 1024 * 1024,
            disable_semaphore_checks=True,
        ),
        name="gated_mix_decode",
    )(
        A_x.reshape(BATCH, D_MODEL),
        A_k_cache.reshape(STREAMS, WAVES, SEQ, D_HEAD),
        A_v_cache.reshape(STREAMS, WAVES, SEQ, D_HEAD),
        A_wq,
        A_wo,
        B_w_gate.T,
        B_w_up.T,
        B_w_down,
        gate_w.reshape(D_MODEL // 128, 128),
    )
    return out.reshape(BATCH, 1, D_MODEL)
```

```python
import functools

import jax
import jax.experimental.pallas as pl
import jax.experimental.pallas.tpu as pltpu
import jax.numpy as jnp
import numpy as np
from jax import lax

BATCH, D_MODEL, HEADS, SEQ, D_HEAD, D_FF = 4, 512, 32, 4096, 128, 1376

STREAMS = 16
WAVES = BATCH * HEADS // STREAMS
HEAD_GROUPS = STREAMS // BATCH
KEYS = 128
CHUNKS = SEQ // KEYS
STEPS = WAVES * CHUNKS
SLOTS = 6

W_ROWS = 32
FF_BLOCKS = D_FF // W_ROWS
GATE_ROW0 = HEADS * D_HEAD
UP_ROW0 = GATE_ROW0 + D_FF
FF_EDGES = (0,) + tuple(range(D_FF % 128, D_FF + 1, 128))
FF_TILES = tuple(zip(FF_EDGES[:-1], FF_EDGES[1:]))
DOWN_PIECES = ((0, 31), (31, 39), (39, FF_BLOCKS))
DOWN_ALTERNATING = 25
WARMUP_PAIRS = 14

_CONTRACT_LAST = (((1,), (1,)), ((), ()))


def _dot(a, b):
    return jnp.dot(a, b, preferred_element_type=jnp.float32)


def _dot_t(a, b):
    return lax.dot_general(a, b, _CONTRACT_LAST, preferred_element_type=jnp.float32)


def _wait_filled(buf, sem):
    pltpu.make_async_copy(buf, buf, sem).wait()


def _start_rows(src, dst, dst_row0, block, sem, priority):
    def rows(row0):
        return pl.ds(row0 if isinstance(row0, int) else pl.multiple_of(row0, W_ROWS), W_ROWS)

    row0 = block * W_ROWS
    pltpu.make_async_copy(
        src.at[rows(row0), :], dst.at[rows(dst_row0 + row0), :], sem
    ).start(priority=priority)


def _kernel(
    x_hbm, k_hbm, v_hbm, wq_hbm, wo_hbm, wgate_t_hbm, wup_t_hbm, wdown_hbm, gate_w_hbm,
    out_hbm,
    kv_buf, wq_buf, w_buf, wdown_buf, x_buf, gate_w_buf, q_buf, out_buf, sems,
):
    f32, bf16 = jnp.float32, jnp.bfloat16
    x_sem, gate_w_sem, wq_sem, w_sem = (sems.at[i] for i in (0, 1, 2, SLOTS - 1))

    def start_kv(step, slot, n):
        is_v, stream = divmod(n, STREAMS)
        batch, head_group = divmod(stream, HEAD_GROUPS)
        wave = lax.div(step, CHUNKS)
        key0 = pl.multiple_of(lax.rem(step, CHUNKS) * KEYS, KEYS)
        pltpu.make_async_copy(
            (k_hbm, v_hbm)[is_v].at[stream, wave, pl.ds(key0, KEYS), :],
            kv_buf.at[slot, is_v, head_group * BATCH + batch],
            sems.at[slot],
        ).start(priority=1 - n % 2)

    def projection_copies(i, _, warmup_pairs=0):
        for j in range(8):
            block = j * 16 + i
            rows = pl.ds(pl.multiple_of(lax.div(block, 2) * 8, 8), 8)
            cols = pl.ds(pl.multiple_of(lax.rem(block, 2) * 2048, 2048), 2048)
            pltpu.make_async_copy(
                wq_hbm.at[rows, cols], wq_buf.at[rows, cols], wq_sem
            ).start(priority=1)
            _start_rows(wo_hbm, w_buf, 0, block, w_sem, int(j < warmup_pairs))

    projection_copies(jnp.int32(0), None, WARMUP_PAIRS)
    projection_copies(jnp.int32(1), None, WARMUP_PAIRS - 8)
    lax.fori_loop(2, 16, projection_copies, None)

    x_copy = pltpu.make_async_copy(x_hbm, x_buf, x_sem)
    gate_w_copy = pltpu.make_async_copy(gate_w_hbm, gate_w_buf, gate_w_sem)
    x_copy.start()
    gate_w_copy.start()

    def ffn_copies(i, _):
        block = lax.rem(i * 18, FF_BLOCKS)
        _start_rows(wgate_t_hbm, w_buf, GATE_ROW0, block, w_sem, 1)
        _start_rows(wup_t_hbm, w_buf, UP_ROW0, block, w_sem, 0)

    lax.fori_loop(0, FF_BLOCKS, ffn_copies, None)

    x_copy.wait()
    gate_w_copy.wait()
    row = lax.broadcasted_iota(jnp.int32, (STREAMS, D_HEAD), 0)
    head_group = row >> 2
    batch = lax.broadcasted_iota(jnp.int32, (STREAMS, D_MODEL), 0) & (BATCH - 1)
    x = x_buf[...].astype(f32)
    x_rows = jnp.broadcast_to(x[0:1], (STREAMS, D_MODEL))
    for b in range(1, BATCH):
        x_rows = jnp.where(batch == b, jnp.broadcast_to(x[b:b + 1], x_rows.shape), x_rows)
    x_rows_bf16 = x_rows.astype(bf16)

    gate_w = gate_w_buf[...].astype(f32)
    gate_terms = x_rows[:, 0:128] * gate_w[0:1]
    for j in range(1, D_MODEL // 128):
        gate_terms = gate_terms + x_rows[:, j * 128:(j + 1) * 128] * gate_w[j:j + 1]
    gate = jax.nn.sigmoid(jnp.sum(gate_terms, axis=-1, keepdims=True))

    def fill_slot(step, _):
        for n in range(2 * STREAMS):
            start_kv(step, step, n)

    def fill_slot_and_project(step, _):
        fill_slot(step, None)
        for u in range(2):
            wave = 2 * step + u
            q = None
            for j in range(HEAD_GROUPS):
                cols = pl.ds(pl.multiple_of((j * WAVES + wave) * D_HEAD, D_HEAD), D_HEAD)
                q_j = _dot(x_rows_bf16, wq_buf[:, cols])
                q = q_j if q is None else jnp.where(head_group == j, q_j, q)
            q_buf[wave] = q.astype(bf16)

    _wait_filled(wq_buf, wq_sem)
    lax.fori_loop(0, WAVES // 2, fill_slot_and_project, None)
    lax.fori_loop(WAVES // 2, SLOTS - 1, fill_slot, None)

    _wait_filled(w_buf, w_sem)
    hidden = []
    for lo, hi in FF_TILES:
        g = _dot_t(x_rows_bf16, w_buf[GATE_ROW0 + lo:GATE_ROW0 + hi, :])
        u = _dot_t(x_rows_bf16, w_buf[UP_ROW0 + lo:UP_ROW0 + hi, :])
        hidden.append((g * jax.nn.sigmoid(g) * u).astype(bf16))

    lowest = np.finfo(np.float32).min

    def attend(step, carry, prefetch):
        slot, free_slot, m, l, acc, attn = carry
        wave = lax.div(step, CHUNKS)
        _wait_filled(kv_buf.at[slot], sems.at[slot])

        q = q_buf[wave]
        s = None
        for r in range(STREAMS):
            if prefetch:
                start_kv(step + SLOTS - 1, free_slot, r)
            s_r = _dot_t(q, kv_buf[slot, 0, r])
            s = s_r if s is None else jnp.where(row == r, s_r, s)
        s = s * np.float32(D_HEAD ** -0.5)

        m_new = jnp.maximum(m, jnp.max(s, axis=-1, keepdims=True))
        alpha = jnp.exp(m - m_new)
        p = jnp.exp(s - m_new)
        l = alpha * l + p
        p = p.astype(bf16)

        pv = None
        for r in range(STREAMS):
            if prefetch:
                start_kv(step + SLOTS - 1, free_slot, STREAMS + r)
            pv_r = _dot(p, kv_buf[slot, 1, r])
            pv = pv_r if pv is None else jnp.where(row == r, pv_r, pv)
        acc = alpha * acc + pv

        def finish_wave(m, l, acc, attn):
            o = acc / jnp.sum(l, axis=-1, keepdims=True)
            for j in range(HEAD_GROUPS):
                rows = pl.ds(pl.multiple_of((j * WAVES + wave) * D_HEAD, D_HEAD), D_HEAD)
                o_j = jnp.where(head_group == j, o, 0.0).astype(bf16)
                attn = attn + _dot(o_j, w_buf[rows, :])
            return jnp.full_like(m, lowest), jnp.zeros_like(l), jnp.zeros_like(acc), attn

        state = lax.cond(
            lax.rem(step, CHUNKS) == CHUNKS - 1,
            finish_wave, lambda *state: state, m_new, l, acc, attn,
        )
        next_slot = jnp.where(slot == SLOTS - 1, 0, slot + 1)
        return (next_slot, slot) + tuple(state)

    carry = (
        jnp.int32(0),
        jnp.int32(SLOTS - 1),
        jnp.full((STREAMS, 1), lowest, f32),
        jnp.zeros((STREAMS, D_HEAD), f32),
        jnp.zeros((STREAMS, D_HEAD), f32),
        jnp.zeros((STREAMS, D_MODEL), f32),
    )
    last_prefetch = STEPS - (SLOTS - 1)
    carry = lax.fori_loop(0, last_prefetch, functools.partial(attend, prefetch=True), carry)

    down_sems = [sems.at[i] for i in ((last_prefetch - 1) % SLOTS, SLOTS, SLOTS + 1)]
    for (lo, hi), sem in zip(DOWN_PIECES, down_sems):
        for n in range(lo, hi):
            if n < DOWN_ALTERNATING:
                _start_rows(wdown_hbm, wdown_buf, 0, n * 9 % DOWN_ALTERNATING, sem, 1 - n % 2)
            else:
                _start_rows(wdown_hbm, wdown_buf, 0, n, sem, 1)

    carry = lax.fori_loop(last_prefetch, STEPS, functools.partial(attend, prefetch=False), carry)

    attn = carry[-1]
    attn = attn[0:8] + attn[8:16]
    attn = attn + pltpu.roll(attn, BATCH, 0)

    ffn = None
    for (lo, hi), sem in zip(DOWN_PIECES, down_sems):
        _wait_filled(wdown_buf.at[pl.ds(lo * W_ROWS, (hi - lo) * W_ROWS), :], sem)
        for h, (r0, r1) in zip(hidden, FF_TILES):
            if lo * W_ROWS <= r0 and r1 <= hi * W_ROWS:
                part = _dot(h, wdown_buf[r0:r1, :])
                ffn = part if ffn is None else ffn + part

    out = gate[0:8] * attn + (1.0 - gate[0:8]) * ffn[0:8]
    out_buf[...] = out[0:BATCH].astype(bf16)
    out_copy = pltpu.make_async_copy(out_buf, out_hbm, sems.at[0])
    out_copy.start()
    out_copy.wait()


@jax.jit
def pallas_gated_mix__mha_block_cached__swiglu_ffn__decode_kernel(
    A_x: jax.Array,
    A_k_cache: jax.Array,
    A_v_cache: jax.Array,
    A_wq: jax.Array,
    A_wo: jax.Array,
    B_x: jax.Array,
    B_w_gate: jax.Array,
    B_w_up: jax.Array,
    B_w_down: jax.Array,
    gate_w: jax.Array,
):
    del B_x
    bf16 = jnp.bfloat16
    hbm = pl.BlockSpec(memory_space=pltpu.HBM)
    out = pl.pallas_call(
        _kernel,
        out_shape=jax.ShapeDtypeStruct((BATCH, D_MODEL), bf16),
        in_specs=[hbm] * 9,
        out_specs=hbm,
        scratch_shapes=[
            pltpu.VMEM((SLOTS, 2, STREAMS, KEYS, D_HEAD), bf16),
            pltpu.VMEM((D_MODEL, HEADS * D_HEAD), bf16),
            pltpu.VMEM((UP_ROW0 + D_FF, D_MODEL), bf16),
            pltpu.VMEM((D_FF, D_MODEL), bf16),
            pltpu.VMEM((BATCH, D_MODEL), bf16),
            pltpu.VMEM((D_MODEL // 128, 128), bf16),
            pltpu.VMEM((WAVES, STREAMS, D_HEAD), bf16),
            pltpu.VMEM((BATCH, D_MODEL), bf16),
            pltpu.SemaphoreType.DMA((SLOTS + 2,)),
        ],
        compiler_params=pltpu.CompilerParams(vmem_limit_bytes=32 * 1024 * 1024),
        name="gated_mix_decode",
    )(
        A_x.reshape(BATCH, D_MODEL),
        A_k_cache.reshape(STREAMS, WAVES, SEQ, D_HEAD),
        A_v_cache.reshape(STREAMS, WAVES, SEQ, D_HEAD),
        A_wq,
        A_wo,
        B_w_gate.T,
        B_w_up.T,
        B_w_down,
        gate_w.reshape(D_MODEL // 128, 128),
    )
    return out.reshape(BATCH, 1, D_MODEL)
```
